```python
import os as _os
_os.environ.setdefault("JAX_PLATFORMS", "cpu")
import jax
import jax.numpy as jnp

def _softmax(x, axis=-1):
    return jax.nn.softmax(x, axis=axis)
def _gelu(x):
    return jax.nn.gelu(x, approximate=True)
def _silu(x):
    return jax.nn.silu(x)
def _sigmoid(x):
    return jax.nn.sigmoid(x)
def _layernorm(x, axis=-1, eps=1e-5):
    m = jnp.mean(x, axis=axis, keepdims=True)
    v = jnp.var(x, axis=axis, keepdims=True)
    return (x - m) / jnp.sqrt(v + eps)
def _scatter_add(tgt, idx, src, axis=0):
    return tgt.at[idx].add(src)
def _segment_sum(src, seg, n):
    return jax.ops.segment_sum(src, seg, n)
class _Rng:
    def __init__(self, key):
        self._k = key
    def _next(self):
        self._k, sub = jax.random.split(self._k)
        return sub
    def normal(self, shape):
        return jax.random.normal(self._next(), shape, dtype=jnp.bfloat16)
    def randint(self, lo, hi, shape):
        return jax.random.randint(self._next(), shape, lo, hi, dtype=jnp.int32)
    def uniform(self, shape, lo=0.0, hi=1.0):
        return jax.random.uniform(self._next(), shape, jnp.bfloat16, lo, hi)
    def permutation(self, n):
        return jax.random.permutation(self._next(), n)


kernel_name = 'standalone__gqa_block_cached__near_ridge'

def setup_inputs():
    _rng = _Rng(jax.random.key(int.from_bytes(__import__("os").urandom(4), "little")))
    _w = (lambda a: (lambda t: t.astype(jnp.bfloat16) if jnp.issubdtype(t.dtype, jnp.floating) else t)(jnp.asarray(a)))
    B, Sq, D = 8, 96, 640
    Hq, Hkv, Sk, Dh = 32, 32, 512, 128
    assert Hq % Hkv == 0, (Hq, Hkv)
    return {
        "x": _w((lambda *s: _rng.normal(s) * 0.2)(B, Sq, D)),
        "k_cache": _w((lambda *s: _rng.normal(s) * 3.2)(B, Hkv, Sk, Dh)),
        "v_cache": _w((lambda *s: _rng.normal(s) * 0.05)(B, Hkv, Sk, Dh)),
        "wq": _w((lambda *s: _rng.normal(s) * 0.2)(D, Hq * Dh) * (D ** -0.5)),
        "wo": _w((lambda *s: _rng.normal(s) * 0.05)(Hq * Dh, D) * ((Hq * Dh) ** -0.5)),
    }

def reference(x, k_cache, v_cache, wq, wo):
    B, Sq, D = x.shape
    Hq, Dh = 32, 128
    Hkv = k_cache.shape[1]
    rep = Hq // Hkv
    q = (lambda x, *d: x.transpose(*d))((x @ wq).reshape(B, Sq, Hq, Dh), 0, 2, 1, 3)
    k = jnp.repeat(k_cache, rep, axis=1)
    v = jnp.repeat(v_cache, rep, axis=1)
    scores = jnp.einsum("bhqd,bhkd->bhqk", q, k) * (Dh ** -0.5)
    p = _softmax(scores, axis=-1)
    o = jnp.einsum("bhqk,bhkd->bhqd", p, v)
    return (lambda x, *d: x.transpose(*d))(o, 0, 2, 1, 3).reshape(B, Sq, Hq * Dh) @ wo
```

```python
import functools

import jax
import jax.numpy as jnp
import jax.experimental.pallas as pl
import jax.experimental.pallas.tpu as pltpu


def _kernel(x_ref, k_ref, v_ref, wq_ref, wo_ref, o_ref, acc_ref, *, B, Sq, Dh, scale):
    h = pl.program_id(0)

    @pl.when(h == 0)
    def _():
        acc_ref[...] = jnp.zeros_like(acc_ref)

    q = jnp.dot(x_ref[...], wq_ref[...], preferred_element_type=jnp.float32)
    q = (q * scale).astype(jnp.bfloat16)

    outs = []
    for b in range(B):
        qb = q[b * Sq:(b + 1) * Sq, :]
        kb = k_ref[b, 0]
        vb = v_ref[b, 0]
        s = jax.lax.dot_general(qb, kb, (((1,), (1,)), ((), ())),
                                preferred_element_type=jnp.float32)
        m = jnp.max(s, axis=-1, keepdims=True)
        p = jnp.exp(s - m)
        l = jnp.sum(p, axis=-1, keepdims=True)
        ob = jnp.dot(p.astype(jnp.bfloat16), vb, preferred_element_type=jnp.float32)
        ob = ob * (1.0 / l)
        outs.append(ob.astype(jnp.bfloat16))
    o = jnp.concatenate(outs, axis=0)
    acc_ref[...] += jnp.dot(o, wo_ref[...], preferred_element_type=jnp.float32)

    @pl.when(h == pl.num_programs(0) - 1)
    def _():
        o_ref[...] = acc_ref[...].astype(o_ref.dtype)


@jax.jit
def pallas_standalone__gqa_block_cached__near_ridge_kernel(
    x: jax.Array,
    k_cache: jax.Array,
    v_cache: jax.Array,
    wq: jax.Array,
    wo: jax.Array,
):
    B, Sq, D = x.shape
    _, H, Sk, Dh = k_cache.shape
    M = B * Sq
    x2 = x.reshape(M, D)

    kernel = functools.partial(_kernel, B=B, Sq=Sq, Dh=Dh, scale=float(Dh) ** -0.5)
    out = pl.pallas_call(
        kernel,
        grid=(H,),
        in_specs=[
            pl.BlockSpec((M, D), lambda h: (0, 0)),
            pl.BlockSpec((B, 1, Sk, Dh), lambda h: (0, h, 0, 0)),
            pl.BlockSpec((B, 1, Sk, Dh), lambda h: (0, h, 0, 0)),
            pl.BlockSpec((D, Dh), lambda h: (0, h)),
            pl.BlockSpec((Dh, D), lambda h: (h, 0)),
        ],
        out_specs=pl.BlockSpec((M, D), lambda h: (0, 0)),
        out_shape=jax.ShapeDtypeStruct((M, D), x.dtype),
        scratch_shapes=[pltpu.VMEM((M, D), jnp.float32)],
        compiler_params=pltpu.CompilerParams(
            dimension_semantics=("arbitrary",),
            vmem_limit_bytes=64 * 1024 * 1024,
        ),
    )(x2, k_cache, v_cache, wq, wo)
    return out.reshape(B, Sq, D)
```

```python
import functools

import jax
import jax.numpy as jnp
import jax.experimental.pallas as pl
import jax.experimental.pallas.tpu as pltpu

_NBUF = 2


def _kernel(x_ref, k_hbm, v_hbm, wq_ref, wo_ref, o_hbm,
            acc_ref, kbuf, vbuf, obuf, kv_sems, o_sems, *, B, Sq, scale):
    h = pl.program_id(0)
    H = pl.num_programs(0)

    def kcopy(hh, slot):
        return pltpu.make_async_copy(k_hbm.at[:, hh], kbuf.at[slot], kv_sems.at[0, slot])

    def vcopy(hh, slot):
        return pltpu.make_async_copy(v_hbm.at[:, hh], vbuf.at[slot], kv_sems.at[1, slot])

    def ocopy(b):
        rows = pl.ds(b * Sq, Sq)
        return pltpu.make_async_copy(obuf.at[rows], o_hbm.at[rows], o_sems.at[b])

    def start_head(hh, slot):
        kcopy(hh, slot).start()
        vcopy(hh, slot).start()

    @pl.when(h == 0)
    def _():
        for j in range(_NBUF - 1):
            start_head(j, j)
        acc_ref[...] = jnp.zeros_like(acc_ref)

    nxt = h + (_NBUF - 1)

    @pl.when(nxt < H)
    def _():
        start_head(nxt, nxt % _NBUF)

    slot = h % _NBUF

    def body(last):
        wq = wq_ref[...]
        wo = wo_ref[...]
        qs = []
        for b in range(B):
            qb = jnp.dot(x_ref[b * Sq:(b + 1) * Sq, :], wq,
                         preferred_element_type=jnp.float32)
            qs.append((qb * scale).astype(jnp.bfloat16))

        kcopy(h, slot).wait()
        vcopy(h, slot).wait()

        def qk(b):
            return jax.lax.dot_general(qs[b], kbuf[slot, b], (((1,), (1,)), ((), ())),
                                       preferred_element_type=jnp.float32)

        def pv(b, s):
            m = jnp.max(s, axis=-1, keepdims=True)
            p = jnp.exp(s - m)
            l = jnp.sum(p, axis=-1, keepdims=True)
            ob = jnp.dot(p.astype(jnp.bfloat16), vbuf[slot, b],
                         preferred_element_type=jnp.float32)
            return (ob * (1.0 / l)).astype(jnp.bfloat16)

        def oproj(b, o):
            r = acc_ref[b * Sq:(b + 1) * Sq, :] + jnp.dot(
                o, wo, preferred_element_type=jnp.float32)
            if last:
                obuf[b * Sq:(b + 1) * Sq, :] = r.astype(obuf.dtype)
                ocopy(b).start()
            else:
                acc_ref[b * Sq:(b + 1) * Sq, :] = r

        s, o = {}, {}
        for i in range(-1, B + 1):
            if 0 <= i + 1 < B:
                s[i + 1] = qk(i + 1)
            if 0 <= i < B:
                o[i] = pv(i, s.pop(i))
            if 0 <= i - 1 < B:
                oproj(i - 1, o.pop(i - 1))

        if last:
            for b in range(B):
                ocopy(b).wait()

    @pl.when(h < H - 1)
    def _():
        body(False)

    @pl.when(h == H - 1)
    def _():
        body(True)


@jax.jit
def pallas_standalone__gqa_block_cached__near_ridge_kernel(
    x: jax.Array,
    k_cache: jax.Array,
    v_cache: jax.Array,
    wq: jax.Array,
    wo: jax.Array,
):
    B, Sq, D = x.shape
    _, H, Sk, Dh = k_cache.shape
    M = B * Sq
    x2 = x.reshape(M, D)

    kernel = functools.partial(_kernel, B=B, Sq=Sq, scale=float(Dh) ** -0.5)
    out = pl.pallas_call(
        kernel,
        grid=(H,),
        in_specs=[
            pl.BlockSpec((M, D), lambda h: (0, 0)),
            pl.BlockSpec(memory_space=pl.ANY),
            pl.BlockSpec(memory_space=pl.ANY),
            pl.BlockSpec((D, Dh), lambda h: (0, h)),
            pl.BlockSpec((Dh, D), lambda h: (h, 0)),
        ],
        out_specs=pl.BlockSpec(memory_space=pl.ANY),
        out_shape=jax.ShapeDtypeStruct((M, D), x.dtype),
        scratch_shapes=[
            pltpu.VMEM((M, D), jnp.float32),
            pltpu.VMEM((_NBUF, B, Sk, Dh), k_cache.dtype),
            pltpu.VMEM((_NBUF, B, Sk, Dh), v_cache.dtype),
            pltpu.VMEM((M, D), x.dtype),
            pltpu.SemaphoreType.DMA((2, _NBUF)),
            pltpu.SemaphoreType.DMA((B,)),
        ],
        compiler_params=pltpu.CompilerParams(
            dimension_semantics=("arbitrary",),
            vmem_limit_bytes=64 * 1024 * 1024,
        ),
    )(x2, k_cache, v_cache, wq, wo)
    return out.reshape(B, Sq, D)
```

```python
import functools

import jax
import jax.numpy as jnp
import jax.experimental.pallas as pl
import jax.experimental.pallas.tpu as pltpu

_NBUF = 2


def _kernel(x_ref, k_hbm, v_hbm, wq_ref, wo_ref, o_hbm,
            acc_ref, kbuf, vbuf, obuf, kv_sems, o_sems, *, B, Sq, rep, scale):
    h = pl.program_id(0)
    H = pl.num_programs(0)

    def kv_head(hh):
        return hh if rep == 1 else hh // rep

    def kcopy(hh, slot):
        return pltpu.make_async_copy(k_hbm.at[:, kv_head(hh)], kbuf.at[slot],
                                     kv_sems.at[0, slot])

    def vcopy(hh, slot):
        return pltpu.make_async_copy(v_hbm.at[:, kv_head(hh)], vbuf.at[slot],
                                     kv_sems.at[1, slot])

    def ocopy(b):
        rows = pl.ds(b * Sq, Sq)
        return pltpu.make_async_copy(obuf.at[rows], o_hbm.at[rows], o_sems.at[b])

    def start_head(hh, slot):
        kcopy(hh, slot).start()
        vcopy(hh, slot).start()

    @pl.when(h == 0)
    def _():
        for j in range(_NBUF - 1):
            start_head(j, j)
        acc_ref[...] = jnp.zeros_like(acc_ref)

    nxt = h + (_NBUF - 1)

    @pl.when(nxt < H)
    def _():
        start_head(nxt, nxt % _NBUF)

    slot = h % _NBUF

    def body(last):
        wq = wq_ref[...]
        wo = wo_ref[...]
        qs = []
        for b in range(B):
            qb = jnp.dot(x_ref[b * Sq:(b + 1) * Sq, :], wq,
                         preferred_element_type=jnp.float32)
            qs.append((qb * scale).astype(jnp.bfloat16))

        kcopy(h, slot).wait()
        vcopy(h, slot).wait()

        def qk(b):
            return jax.lax.dot_general(qs[b], kbuf[slot, b], (((1,), (1,)), ((), ())),
                                       preferred_element_type=jnp.float32)

        def pv(b, s):
            m = jnp.max(s, axis=-1, keepdims=True)
            p = jnp.exp(s - m)
            l = jnp.sum(p, axis=-1, keepdims=True)
            ob = jnp.dot(p.astype(jnp.bfloat16), vbuf[slot, b],
                         preferred_element_type=jnp.float32)
            return (ob * (1.0 / l)).astype(jnp.bfloat16)

        def oproj(b, o):
            r = acc_ref[b * Sq:(b + 1) * Sq, :] + jnp.dot(
                o, wo, preferred_element_type=jnp.float32)
            if last:
                obuf[b * Sq:(b + 1) * Sq, :] = r.astype(obuf.dtype)
                ocopy(b).start()
            else:
                acc_ref[b * Sq:(b + 1) * Sq, :] = r

        s, o = {}, {}
        for i in range(-1, B + 1):
            if 0 <= i + 1 < B:
                s[i + 1] = qk(i + 1)
            if 0 <= i < B:
                o[i] = pv(i, s.pop(i))
            if 0 <= i - 1 < B:
                oproj(i - 1, o.pop(i - 1))

        if last:
            for b in range(B):
                ocopy(b).wait()

    @pl.when(h < H - 1)
    def _():
        body(False)

    @pl.when(h == H - 1)
    def _():
        body(True)


@jax.jit
def pallas_standalone__gqa_block_cached__near_ridge_kernel(
    x: jax.Array,
    k_cache: jax.Array,
    v_cache: jax.Array,
    wq: jax.Array,
    wo: jax.Array,
):
    B, Sq, D = x.shape
    _, Hkv, Sk, Dh = k_cache.shape
    H = wq.shape[1] // Dh
    M = B * Sq
    x2 = x.reshape(M, D)

    kernel = functools.partial(_kernel, B=B, Sq=Sq, rep=H // Hkv,
                               scale=float(Dh) ** -0.5)
    out = pl.pallas_call(
        kernel,
        grid=(H,),
        in_specs=[
            pl.BlockSpec((M, D), lambda h: (0, 0)),
            pl.BlockSpec(memory_space=pl.ANY),
            pl.BlockSpec(memory_space=pl.ANY),
            pl.BlockSpec((D, Dh), lambda h: (0, h)),
            pl.BlockSpec((Dh, D), lambda h: (h, 0)),
        ],
        out_specs=pl.BlockSpec(memory_space=pl.ANY),
        out_shape=jax.ShapeDtypeStruct((M, D), x.dtype),
        scratch_shapes=[
            pltpu.VMEM((M, D), jnp.float32),
            pltpu.VMEM((_NBUF, B, Sk, Dh), k_cache.dtype),
            pltpu.VMEM((_NBUF, B, Sk, Dh), v_cache.dtype),
            pltpu.VMEM((M, D), x.dtype),
            pltpu.SemaphoreType.DMA((2, _NBUF)),
            pltpu.SemaphoreType.DMA((B,)),
        ],
        compiler_params=pltpu.CompilerParams(
            dimension_semantics=("arbitrary",),
            vmem_limit_bytes=64 * 1024 * 1024,
        ),
    )(x2, k_cache, v_cache, wq, wo)
    return out.reshape(B, Sq, D)
```
